```python
import os as _os
_os.environ.setdefault("JAX_PLATFORMS", "cpu")
import jax
import jax.numpy as jnp

def _softmax(x, axis=-1):
    return jax.nn.softmax(x, axis=axis)
def _gelu(x):
    return jax.nn.gelu(x, approximate=True)
def _silu(x):
    return jax.nn.silu(x)
def _sigmoid(x):
    return jax.nn.sigmoid(x)
def _layernorm(x, axis=-1, eps=1e-5):
    m = jnp.mean(x, axis=axis, keepdims=True)
    v = jnp.var(x, axis=axis, keepdims=True)
    return (x - m) / jnp.sqrt(v + eps)
def _scatter_add(tgt, idx, src, axis=0):
    return tgt.at[idx].add(src)
def _segment_sum(src, seg, n):
    return jax.ops.segment_sum(src, seg, n)
class _Rng:
    def __init__(self, key):
        self._k = key
    def _next(self):
        self._k, sub = jax.random.split(self._k)
        return sub
    def normal(self, shape):
        return jax.random.normal(self._next(), shape, dtype=jnp.bfloat16)
    def randint(self, lo, hi, shape):
        return jax.random.randint(self._next(), shape, lo, hi, dtype=jnp.int32)
    def uniform(self, shape, lo=0.0, hi=1.0):
        return jax.random.uniform(self._next(), shape, jnp.bfloat16, lo, hi)
    def permutation(self, n):
        return jax.random.permutation(self._next(), n)


kernel_name = 'concat_heads__linear_kernel_hedgehog__ssm_conv_s5__prompt'

def setup_inputs():
    _rng = _Rng(jax.random.key(int.from_bytes(__import__("os").urandom(4), "little")))
    _w = (lambda a: (lambda t: t.astype(jnp.bfloat16) if jnp.issubdtype(t.dtype, jnp.floating) else t)(jnp.asarray(a)))
    def _A_setup():
        B, S, D, H = 1, 2048, 640, 32
        Dh = D // H
        return {
            "x": _w((lambda *s: _rng.normal(s) * 0.4)(B, S, D)),
            "wqkv": _w((lambda *s: _rng.normal(s) * 0.4)(D, 3 * D)),
            "w_phi": _w((lambda *s: _rng.normal(s) * 0.4)(H, Dh, Dh) * (Dh ** -0.5)),
            "wo": _w((lambda *s: _rng.normal(s) * 0.05)(D, D)),
        }
    _A_in = _A_setup()

    def _B_setup():
        B, S, D = 1, 2048, 640
        P = D
        Lambda_re = -0.5 * jnp.exp((lambda *s: _rng.normal(s) * 0.8)(P))
        Lambda_im = (lambda *s: _rng.normal(s) * 0.8)(P) * 1.0
        B_re = (lambda *s: _rng.normal(s) * 0.8)(P, D) * (D ** -0.5)
        B_im = (lambda *s: _rng.normal(s) * 0.8)(P, D) * (D ** -0.5)
        C_re = (lambda *s: _rng.normal(s) * 0.8)(D, P) * (P ** -0.5)
        C_im = (lambda *s: _rng.normal(s) * 0.8)(D, P) * (P ** -0.5)
        log_dt = (lambda *s: _rng.normal(s) * 0.8)(P) * 0.3 - 2.0
        Dskip = (lambda *s: _rng.normal(s) * 0.8)(D)
        return {
            "x": _w((lambda *s: _rng.normal(s) * 0.05)(B, S, D)),
            "Lambda_re": _w(Lambda_re),
            "Lambda_im": _w(Lambda_im),
            "B_re": _w(B_re),
            "B_im": _w(B_im),
            "C_re": _w(C_re),
            "C_im": _w(C_im),
            "log_dt": _w(log_dt),
            "Dskip": _w(Dskip),
        }
    _B_in = _B_setup()

    return {
        "A_x": _A_in["x"],
        "A_wqkv": _A_in["wqkv"],
        "A_w_phi": _A_in["w_phi"],
        "A_wo": _A_in["wo"],
        "B_x": _B_in["x"],
        "B_Lambda_re": _B_in["Lambda_re"],
        "B_Lambda_im": _B_in["Lambda_im"],
        "B_B_re": _B_in["B_re"],
        "B_B_im": _B_in["B_im"],
        "B_C_re": _B_in["C_re"],
        "B_C_im": _B_in["C_im"],
        "B_log_dt": _B_in["log_dt"],
        "B_Dskip": _B_in["Dskip"],
    }

def reference(A_x, A_wqkv, A_w_phi, A_wo, B_x, B_Lambda_re, B_Lambda_im, B_B_re, B_B_im, B_C_re, B_C_im, B_log_dt, B_Dskip):
    def _A_ref(x, wqkv, w_phi, wo):
        B, S, D = x.shape
        H = 32; Dh = D // H
        qkv = (lambda x, *d: x.transpose(*d))((x @ wqkv).reshape(B, S, 3, H, Dh), 2, 0, 3, 1, 4)
        q, k, v = qkv[0], qkv[1], qkv[2]
        pq = jnp.einsum("bhsd,hdf->bhsf", q, w_phi)
        pk = jnp.einsum("bhsd,hdf->bhsf", k, w_phi)
        phi_q = jnp.concatenate([_softmax(pq, axis=-1), _softmax(-pq, axis=-1)], axis=-1)
        phi_k = jnp.concatenate([_softmax(pk, axis=-1), _softmax(-pk, axis=-1)], axis=-1)
        kv = jnp.einsum("bhsf,bhsd->bhfd", phi_k, v)
        z  = jnp.einsum("bhsf->bhf", phi_k)
        num = jnp.einsum("bhqf,bhfd->bhqd", phi_q, kv)
        den = jnp.einsum("bhqf,bhf->bhq", phi_q, z)[..., None] + 1e-6
        o = num / den
        return (lambda x, *d: x.transpose(*d))(o, 0, 2, 1, 3).reshape(B, S, D) @ wo

    def _B_ref(x, Lambda_re, Lambda_im, B_re, B_im, C_re, C_im, log_dt, Dskip):
        Bsz, L, H = x.shape
        Lam = Lambda_re + 1j * Lambda_im
        Bmat = B_re + 1j * B_im
        Cmat = C_re + 1j * C_im
        dt = jnp.exp(log_dt)
        Lam_bar = jnp.exp(dt * Lam)
        B_bar = ((Lam_bar - 1.0) / Lam)[:, None] * Bmat
        Bu = jnp.einsum("bld,pd->blp", x + 0j, B_bar)
        h = jnp.zeros_like(Bu[:, 0, :])
        hs = []
        for t in range(L):
            h = Lam_bar[None, :] * h + Bu[:, t, :]
            hs.append(h)
        hseq = jnp.stack(hs, 1)
        y = 2.0 * jnp.einsum("blp,dp->bld", hseq, Cmat).real + x * Dskip[None, None, :]
        return y

    a = _A_ref(A_x, A_wqkv, A_w_phi, A_wo)
    b = _B_ref(B_x, B_Lambda_re, B_Lambda_im, B_B_re, B_B_im, B_C_re, B_C_im, B_log_dt, B_Dskip)
    return jnp.concatenate([a, b], axis=-1)
```

```python
import jax
import jax.numpy as jnp
from jax import lax
import jax.experimental.pallas as pl
import jax.experimental.pallas.tpu as pltpu

S, D, H, DH = 2048, 640, 32, 20
G = H // 2
TB = 256
LAG = 4
NB = S // TB
ORDER = 'kbqivsczd'
NC = 8
T = TB // NC
TP = T + 4
NL = D // 128
LOG2E = 1.4426950408889634
f32, bf16, i32 = jnp.float32, jnp.bfloat16, jnp.int32

BANDS = ((0, 160), (112, 288), (240, 400), (352, 528), (480, 640))


def _nt(a, b):
    return lax.dot_general(a, b, (((1,), (1,)), ((), ())), preferred_element_type=f32)


def _nn(a, b):
    return lax.dot_general(a, b, (((1,), (0,)), ((), ())), preferred_element_type=f32)


def _rcp(x):
    r = pl.reciprocal(x, approx=True)
    return r * (2.0 - x * r)


def _cmul(ar, ai, br, bi):
    return ar * br - ai * bi, ar * bi + ai * br


def _dual_softmax(p):
    tb = p.shape[1]
    p = p.reshape(G, 5, 8, tb)
    mx = jnp.max(p, axis=1)
    mn = jnp.min(p, axis=1)
    mx = jnp.maximum(mx, pltpu.roll(mx, 4, 1))
    mx = jnp.maximum(mx, pltpu.roll(mx, 2, 1))
    mn = jnp.minimum(mn, pltpu.roll(mn, 4, 1))
    mn = jnp.minimum(mn, pltpu.roll(mn, 2, 1))
    ep = jnp.exp2(p - mx[:, None])
    en = jnp.exp2(mn[:, None] - p)
    sp = jnp.sum(ep, axis=1)
    sn = jnp.sum(en, axis=1)
    sp = sp + pltpu.roll(sp, 4, 1)
    sp = sp + pltpu.roll(sp, 2, 1)
    sn = sn + pltpu.roll(sn, 4, 1)
    sn = sn + pltpu.roll(sn, 2, 1)
    rp = _rcp(sp)
    rn = _rcp(sn)
    return jnp.concatenate([ep * rp[:, None], en * rn[:, None]], axis=1)


def _kernel(
    xa_hbm, wqkv_hbm, wphi_hbm, wo_hbm, xb_hbm, lre_hbm, lim_hbm, bre_hbm, bim_hbm,
    cre_hbm, cim_hbm, ldt_hbm, dsk_hbm,
    out_hbm,
    xa, xb, wqkv, wphi, wo, bre, bim, cre, cim, lre, lim, ldt, dsk,
    w2, wt, tabs, pwre, pwim, dvec,
    phiq, kvacc, kvb, bu, hst, oa, ob,
    sem_in, sem_xa, sem_xb, sem_oa, sem_ob,
):
    def mk(n, s, d):
        return pltpu.make_async_copy(s, d, sem_in.at[n])
    c_lre, c_lim, c_ldt, c_dsk = mk(0, lre_hbm, lre), mk(1, lim_hbm, lim), mk(2, ldt_hbm, ldt), mk(3, dsk_hbm, dsk)
    c_wphi, c_bre, c_bim, c_wqkv = mk(4, wphi_hbm, wphi), mk(5, bre_hbm, bre), mk(6, bim_hbm, bim), mk(7, wqkv_hbm, wqkv)
    c_cre, c_cim, c_wo = mk(8, cre_hbm, cre), mk(9, cim_hbm, cim), mk(10, wo_hbm, wo)
    cxb = [pltpu.make_async_copy(xb_hbm.at[i], xb.at[i], sem_xb.at[i]) for i in range(NB)]
    cxa = [pltpu.make_async_copy(xa_hbm.at[i], xa.at[i], sem_xa.at[i]) for i in range(NB)]
    c_bre.start()
    cxb[0].start()
    c_bim.start()
    cxb[1].start()
    c_lre.start()
    cxb[2].start()
    c_lim.start()
    c_ldt.start()
    c_dsk.start()
    c_wphi.start()
    c_wqkv.start()
    for i in range(3, LAG + 1):
        cxb[i].start()
    cxa[0].start()
    c_cre.start()
    c_cim.start()
    for i in range(1, NB):
        if i + LAG < NB:
            cxb[i + LAG].start()
        cxa[i].start()
    c_wo.start()

    def bu_proj(i, which, fillers=()):
        fillers = list(fillers)
        b = (bre, bim)[which]
        if not fillers:
            res = _nt(xb[i], b[...])
            for j in range(NL):
                for c in range(NC):
                    bu[i, which * NL + j, TP * c:TP * c + T, :] = res[T * c:T * (c + 1), 128 * j:128 * (j + 1)]
            return
        xbi = xb[i]
        per = -(-len(fillers) // NL)
        for j in range(NL):
            res = _nt(xbi, b[128 * j:128 * (j + 1), :])
            for c in range(NC):
                bu[i, which * NL + j, TP * c:TP * c + T, :] = res[T * c:T * (c + 1), :]
            for f in fillers[per * j:per * (j + 1)]:
                f()

    c_bre.wait()
    cxb[0].wait()
    bu_proj(0, 0)
    kvacc[...] = jnp.zeros(kvacc.shape, f32)
    hst[...] = jnp.zeros(hst.shape, f32)
    w2[...] = jnp.zeros(w2.shape, f32)
    c_bim.wait()
    cxb[1].wait()
    bu_proj(0, 1)
    bu_proj(1, 0)
    bu_proj(1, 1)
    for c in (c_lre, c_lim, c_ldt, c_dsk, c_wphi):
        c.wait()
    cxb[2].wait()
    bu_proj(2, 0)

    l_re = lre[...].reshape(1, D).astype(f32)
    l_im = lim[...].reshape(1, D).astype(f32)
    dt = jnp.exp(ldt[...].reshape(1, D).astype(f32)).astype(bf16).astype(f32)
    dvec[...] = jnp.broadcast_to(dsk[...].reshape(1, D).astype(f32), (8, D))
    zr = dt * l_re
    zi = dt * l_im
    sub = lax.broadcasted_iota(i32, (8, D), 0)
    n = (sub + 1).astype(f32)
    mag = jnp.exp(n * zr)
    pr = mag * jnp.cos(n * zi)
    pi = mag * jnp.sin(n * zi)
    a_re = pr[0:1]
    a_im = pi[0:1]
    tabs[8] = jnp.broadcast_to(a_re, (8, D))
    tabs[9] = jnp.broadcast_to(a_im, (8, D))
    a8r = jnp.broadcast_to(pr[7:8], (8, D))
    a8i = jnp.broadcast_to(pi[7:8], (8, D))
    den = l_re * l_re + l_im * l_im
    nr = a_re - 1.0
    s_r = jnp.broadcast_to(2.0 * (nr * l_re + a_im * l_im) / den, (8, D))
    s_i = jnp.broadcast_to(2.0 * (a_im * l_re - nr * l_im) / den, (8, D))
    tabs[10] = s_r
    tabs[11] = s_i
    for q in range(T // 8):
        tr, ti = _cmul(pr, pi, s_r, s_i)
        pwre[8 * q:8 * q + 8, :] = tr
        pwim[8 * q:8 * q + 8, :] = ti
        if q + 1 < T // 8:
            pr, pi = _cmul(pr, pi, a8r, a8i)
    b1r = jnp.broadcast_to(pr[7:8], (8, D))
    b1i = jnp.broadcast_to(pi[7:8], (8, D))
    b2r, b2i = _cmul(b1r, b1i, b1r, b1i)
    b4r, b4i = _cmul(b2r, b2i, b2r, b2i)
    for k, (vr, vi, lo, hi) in enumerate(((b1r, b1i, 0, 1), (b1r, b1i, 1, 8), (b2r, b2i, 2, 8), (b4r, b4i, 4, 8))):
        keep = (sub >= lo) & (sub < hi)
        tabs[2 * k] = jnp.where(keep, vr, 0.0)
        tabs[2 * k + 1] = jnp.where(keep, vi, 0.0)

    for d in range(DH):
        w2[pl.ds(24 * d, DH), :] = wphi[d].astype(f32)
    hrow = lax.broadcasted_iota(i32, (H, D), 0)
    ccol = lax.broadcasted_iota(i32, (H, D), 1)
    hsel = jnp.where(((ccol * 3277) >> 16) == hrow, 1.0, 0.0).astype(bf16)
    r2 = _nn(w2[...].astype(bf16), hsel)
    c8 = lax.broadcasted_iota(i32, (24, D), 1)
    h8 = (c8 * 3277) >> 16
    d8 = c8 - DH * h8
    wpt = jnp.zeros((24, D), f32)
    for d in range(DH):
        wpt = wpt + jnp.where(d8 == d, r2[24 * d:24 * (d + 1)], 0.0)
    rr = lax.broadcasted_iota(i32, (48, 24), 0)
    ff = lax.broadcasted_iota(i32, (48, 24), 1)
    e40 = jnp.where((4 * (rr >> 3) + ((rr & 7) >> 1)) == ff, 1.0, 0.0).astype(bf16)

    bu_proj(2, 1)
    r40 = _nn(e40, wpt.astype(bf16))
    subp = lax.broadcasted_iota(i32, (8, 128), 0) & 1
    abands = []
    for kt, (r0, r1) in enumerate(BANDS):
        hc = h8[0:8, 128 * kt:128 * (kt + 1)] - subp
        slabs = []
        for q in range(r0 // 8, r1 // 8):
            slabs.append(jnp.where(hc == 2 * (q // 5), r40[8 * (q % 5):8 * (q % 5) + 8, 128 * kt:128 * (kt + 1)], 0.0))
        abands.append(jnp.concatenate(slabs, 0).astype(bf16))

    c_wqkv.wait()
    for i in range(3, LAG + 1):
        cxb[i].wait()
    segs = ((0, 112, 0, None), (112, 160, 0, 1), (160, 240, 1, None), (240, 288, 1, 2), (288, 352, 2, None),
            (352, 400, 2, 3), (400, 480, 3, None), (480, 528, 3, 4), (528, 640, 4, None))
    for part in range(2):
        pieces = [_nt(abands[kt], wqkv[:, part * D + 128 * kt: part * D + 128 * (kt + 1)]) for kt in range(5)]
        for r0, r1, ka, kb in segs:
            v = pieces[ka][r0 - BANDS[ka][0]:r1 - BANDS[ka][0]]
            if kb is not None:
                v = v + pieces[kb][r0 - BANDS[kb][0]:r1 - BANDS[kb][0]]
            wt[part * D + r0:part * D + r1, :] = (v * LOG2E).astype(bf16)
    def wvt(kt, nt):
        def run():
            wt[2 * D + 128 * kt:2 * D + 128 * (kt + 1), 128 * nt:128 * (nt + 1)] = (
                wqkv[128 * nt:128 * (nt + 1), 2 * D + 128 * kt:2 * D + 128 * (kt + 1)].T)
        return run
    tfill = [wvt(kt, nt) for kt in range(5) for nt in range(5)]
    for f in tfill:
        f()
    for i in range(3, LAG + 1):
        bu_proj(i, 0)
        bu_proj(i, 1)
    c_cre.wait()
    c_cim.wait()

    def scan(i):
        hr_all, hi_all = [], []
        for j in range(NL):
            ls = slice(128 * j, 128 * (j + 1))
            ar = tabs[8, :, ls]
            ai = tabs[9, :, ls]
            hr = bu[i, j, pl.ds(0, NC, stride=TP), :]
            hi = bu[i, NL + j, pl.ds(0, NC, stride=TP), :]
            for t in range(1, T):
                ur = bu[i, j, pl.ds(t, NC, stride=TP), :]
                ui = bu[i, NL + j, pl.ds(t, NC, stride=TP), :]
                mr, mi = _cmul(ar, ai, hr, hi)
                hr = mr + ur
                hi = mi + ui
                bu[i, j, pl.ds(t, NC, stride=TP), :] = hr
                bu[i, NL + j, pl.ds(t, NC, stride=TP), :] = hi
            inr = hst[0, :, ls]
            ini = hst[1, :, ls]
            mr, mi = _cmul(tabs[0, :, ls], tabs[1, :, ls], inr, ini)
            er = hr + mr
            ei = hi + mi
            for k, sh in ((1, 1), (2, 2), (3, 4)):
                mr, mi = _cmul(tabs[2 * k, :, ls], tabs[2 * k + 1, :, ls],
                               pltpu.roll(er, sh, 0), pltpu.roll(ei, sh, 0))
                er = er + mr
                ei = ei + mi
            subl = lax.broadcasted_iota(i32, (8, 128), 0)
            cinr = jnp.where(subl == 0, inr, pltpu.roll(er, 1, 0))
            cini = jnp.where(subl == 0, ini, pltpu.roll(ei, 1, 0))
            hst[0, :, ls] = jnp.broadcast_to(er[7:8], (8, 128))
            hst[1, :, ls] = jnp.broadcast_to(ei[7:8], (8, 128))
            pr_ = pwre[:, ls]
            pi_ = pwim[:, ls]
            sr_ = jnp.broadcast_to(tabs[10, 0:1, ls], (T, 128))
            si_ = jnp.broadcast_to(tabs[11, 0:1, ls], (T, 128))
            nsr_ = -sr_
            hrs, his = [], []
            for c in range(NC):
                cr = jnp.broadcast_to(cinr[c:c + 1], (T, 128))
                ci = jnp.broadcast_to(cini[c:c + 1], (T, 128))
                mr, mi = _cmul(pr_, pi_, cr, ci)
                lr = bu[i, j, TP * c:TP * c + T, :]
                li = bu[i, NL + j, TP * c:TP * c + T, :]
                hrs.append((lr * sr_ - li * si_) + mr)
                his.append((li * nsr_ - lr * si_) - mi)
            hr_all.append(jnp.concatenate(hrs, 0))
            hi_all.append(jnp.concatenate(his, 0))
        hre = jnp.concatenate(hr_all, 1).astype(bf16)
        him = jnp.concatenate(hi_all, 1).astype(bf16)
        return hre, him

    def phase1(i, with_bu):
        if with_bu:
            k = i + LAG + 1
            pltpu.make_async_copy(xb_hbm.at[k], xb.at[k], sem_xb.at[k]).wait()
        pltpu.make_async_copy(xa_hbm.at[i], xa.at[i], sem_xa.at[i]).wait()
        xai = xa[i]
        st = {}

        def do_k():
            st['phk'] = _dual_softmax(_nt(wt[D:2 * D, :], xai))

        def do_q():
            phiq[i] = _dual_softmax(_nt(wt[0:D, :], xai)).reshape(2 * D, TB).astype(bf16)

        def do_v():
            st['vt'] = _nt(wt[2 * D:3 * D, :], xai)

        def do_b():
            if with_bu:
                bu_proj(i + LAG + 1, 0)

        def do_i():
            if with_bu:
                bu_proj(i + LAG + 1, 1)

        def do_z():
            ones8 = jnp.ones((8, TB), f32)
            for g in range(G):
                vaug = jnp.concatenate([st['vt'][40 * g:40 * (g + 1)], ones8], axis=0).astype(bf16)
                kvacc[g] += _nt(vaug, st['phk'][g].reshape(80, TB).astype(bf16))

        def do_s():
            st['h'] = scan(i)

        def do_c():
            hre, him = st['h']
            y = _nt(hre, cre[...]) + _nt(him, cim[...])
            ob[i] = y + xb[i].astype(f32) * dvec[0:1, :]

        def do_d():
            pltpu.make_async_copy(ob.at[i], out_hbm.at[0, pl.ds(i * TB, TB), pl.ds(D, D)], sem_ob.at[i]).start()

        for ch in ORDER:
            dict(k=do_k, q=do_q, v=do_v, b=do_b, i=do_i, z=do_z, s=do_s, c=do_c, d=do_d)[ch]()

    NW = NB - LAG - 1
    lax.fori_loop(0, NW, lambda i, c: (phase1(i, True), c)[1], 0)
    lax.fori_loop(NW, NB, lambda i, c: (phase1(i, False), c)[1], 0)

    r3 = lax.broadcasted_iota(i32, (G, 48, 80), 1)
    c3 = lax.broadcasted_iota(i32, (G, 48, 80), 2)
    hh_row = jnp.where(r3 < 40, jnp.where(r3 >= 20, 1, 0), jnp.where(r3 >= 44, 1, 0))
    kvb[...] = jnp.where(hh_row == (c3 & 1), kvacc[...], 0.0).astype(bf16)
    c_wo.wait()

    def numpart(i):
        os_ = []
        for g in range(G):
            r = _nn(kvb[g], phiq[i, 80 * g:80 * (g + 1), :])
            rd = _rcp(r[40:48] + 1e-6)
            r0 = jnp.broadcast_to(rd[0:1], (8, TB))
            r1 = jnp.broadcast_to(rd[4:5], (8, TB))
            os_.append(r[0:40] * jnp.concatenate([r0, r0, rd, r1, r1], 0))
        return jnp.concatenate(os_, 0).astype(bf16)

    ot = numpart(0)
    for i in range(NB):
        ot_next = numpart(i + 1) if i + 1 < NB else None
        oa[i] = lax.dot_general(ot, wo[...], (((0,), (0,)), ((), ())), preferred_element_type=f32)
        pltpu.make_async_copy(oa.at[i], out_hbm.at[0, pl.ds(i * TB, TB), pl.ds(0, D)], sem_oa.at[i]).start()
        ot = ot_next

    for i in range(NB):
        pltpu.make_async_copy(ob.at[i], out_hbm.at[0, pl.ds(i * TB, TB), pl.ds(D, D)], sem_ob.at[i]).wait()
        pltpu.make_async_copy(oa.at[i], out_hbm.at[0, pl.ds(i * TB, TB), pl.ds(0, D)], sem_oa.at[i]).wait()


@jax.jit
def pallas_concat_heads__linear_kernel_hedgehog__ssm_conv_s5__prompt_kernel(A_x, A_wqkv, A_w_phi, A_wo, B_x, B_Lambda_re, B_Lambda_im, B_B_re, B_B_im,
           B_C_re, B_C_im, B_log_dt, B_Dskip):
    any_spec = pl.BlockSpec(memory_space=pl.ANY)
    V = pltpu.VMEM
    scratch = [
        V((NB, TB, D), bf16), V((NB, TB, D), bf16), V((D, 3 * D), bf16), V((DH, DH, H), bf16),
        V((D, D), bf16), V((D, D), bf16), V((D, D), bf16), V((D, D), bf16), V((D, D), bf16),
        V((D,), bf16), V((D,), bf16), V((D,), bf16), V((D,), bf16),
        V((24 * DH, H), f32), V((3 * D, D), bf16),
        V((12, 8, D), f32), V((T, D), f32), V((T, D), f32), V((8, D), f32),
        V((NB, 2 * D, TB), bf16), V((G, 48, 80), f32), V((G, 48, 80), bf16),
        V((NB, 2 * NL, NC * TP, 128), f32), V((2, 8, D), f32),
        V((NB, TB, D), f32), V((NB, TB, D), f32),
        pltpu.SemaphoreType.DMA((11,)), pltpu.SemaphoreType.DMA((NB,)), pltpu.SemaphoreType.DMA((NB,)),
        pltpu.SemaphoreType.DMA((NB,)), pltpu.SemaphoreType.DMA((NB,)),
    ]
    return pl.pallas_call(
        _kernel,
        in_specs=[any_spec] * 13,
        out_specs=any_spec,
        out_shape=jax.ShapeDtypeStruct((1, S, 2 * D), f32),
        scratch_shapes=scratch,
        compiler_params=pltpu.CompilerParams(vmem_limit_bytes=110 * 2 ** 20),
    )(A_x.reshape(NB, TB, D), A_wqkv, jnp.transpose(A_w_phi, (1, 2, 0)), A_wo, B_x.reshape(NB, TB, D),
      B_Lambda_re, B_Lambda_im, B_B_re, B_B_im, B_C_re, B_C_im, B_log_dt, B_Dskip)
```

```python
import jax
import jax.numpy as jnp
from jax import lax
import jax.experimental.pallas as pl
import jax.experimental.pallas.tpu as pltpu

S, D, H, DH = 2048, 640, 32, 20
G = H // 2
TB = 256
NB = S // TB
ORDER = 'kbqivsczd'
NC = 8
T = TB // NC
TP = T + 4
LB = 4
NL = D // 128
LOG2E = 1.4426950408889634
f32, bf16, i32, u32 = jnp.float32, jnp.bfloat16, jnp.int32, jnp.uint32

BANDS = ((0, 160), (112, 288), (240, 400), (352, 528), (480, 640))


def _nt(a, b):
    return lax.dot_general(a, b, (((1,), (1,)), ((), ())), preferred_element_type=f32)


def _nn(a, b):
    return lax.dot_general(a, b, (((1,), (0,)), ((), ())), preferred_element_type=f32)


def _pk(x):
    return pltpu.bitcast(x, u32)


def _up(x):
    return pltpu.bitcast(x, bf16)


def _rcp(x):
    r = pl.reciprocal(x, approx=True)
    return r * (2.0 - x * r)


def _cmul(ar, ai, br, bi):
    return ar * br - ai * bi, ar * bi + ai * br


def _dual_softmax(p):
    tb = p.shape[1]
    p = p.reshape(G, 5, 8, tb)
    mx = jnp.max(p, axis=1)
    mn = jnp.min(p, axis=1)
    mx = jnp.maximum(mx, pltpu.roll(mx, 4, 1))
    mx = jnp.maximum(mx, pltpu.roll(mx, 2, 1))
    mn = jnp.minimum(mn, pltpu.roll(mn, 4, 1))
    mn = jnp.minimum(mn, pltpu.roll(mn, 2, 1))
    ep = jnp.exp2(p - mx[:, None])
    en = jnp.exp2(mn[:, None] - p)
    sp = jnp.sum(ep, axis=1)
    sn = jnp.sum(en, axis=1)
    sp = sp + pltpu.roll(sp, 4, 1)
    sp = sp + pltpu.roll(sp, 2, 1)
    sn = sn + pltpu.roll(sn, 4, 1)
    sn = sn + pltpu.roll(sn, 2, 1)
    rp = _rcp(sp)
    rn = _rcp(sn)
    return jnp.concatenate([ep * rp[:, None], en * rn[:, None]], axis=1)


def _kernel(
    xa_hbm, wqkv_hbm, wphi_hbm, wo_hbm, xb_hbm, lre_hbm, lim_hbm, bre_hbm, bim_hbm,
    cre_hbm, cim_hbm, ldt_hbm, dsk_hbm,
    out_hbm,
    xa, xb, wqkv, wphi, wo, bre, bim, cre, cim, lre, lim, ldt, dsk,
    w2, wt, tabs, pwre, pwim, dvec,
    phiq, kvacc, kvb, bu, hst, oa, ob,
    sem_in, sem_oa, sem_ob,
):
    order = ['lre', 'lim', 'ldt', 'dsk', 'wphi', 'bre', 'xb0', 'xb1', 'bim', 'xb2', 'wqkv']
    order += ['xb%d' % i for i in range(3, LB)] + ['xa0', 'cre', 'cim']
    for i in range(1, NB):
        order += (['xb%d' % (i + LB - 1)] if i + LB - 1 < NB else []) + ['xa%d' % i]
    order += ['wo']
    assert len(set(order)) == len(order) == 11 + 2 * NB
    whole = dict(bre=(bre_hbm, bre), bim=(bim_hbm, bim), lre=(lre_hbm, lre), lim=(lim_hbm, lim),
                 ldt=(ldt_hbm, ldt), dsk=(dsk_hbm, dsk), wphi=(wphi_hbm, wphi), wqkv=(wqkv_hbm, wqkv),
                 cre=(cre_hbm, cre), cim=(cim_hbm, cim), wo=(wo_hbm, wo))
    SEM_XB, SEM_XA = len(whole), len(whole) + NB
    cps = {}
    for n, name in enumerate(whole):
        cps[name] = pltpu.make_async_copy(*whole[name], sem_in.at[n])

    def cp_xb(i):
        return pltpu.make_async_copy(xb_hbm.at[i], xb.at[i], sem_in.at[SEM_XB + i])

    def cp_xa(i):
        return pltpu.make_async_copy(xa_hbm.at[i], xa.at[i], sem_in.at[SEM_XA + i])

    for i in range(NB):
        cps['xb%d' % i] = cp_xb(i)
        cps['xa%d' % i] = cp_xa(i)
    for name in order:
        cps[name].start()
    c_bre, c_bim, c_lre, c_lim, c_ldt, c_dsk = (cps[n] for n in ('bre', 'bim', 'lre', 'lim', 'ldt', 'dsk'))
    c_wphi, c_wqkv, c_cre, c_cim, c_wo = (cps[n] for n in ('wphi', 'wqkv', 'cre', 'cim', 'wo'))
    cxb = [cps['xb%d' % i] for i in range(NB)]
    cxa = [cps['xa%d' % i] for i in range(NB)]

    def bu_proj(i, which):
        res = _nt(xb[i], (bre, bim)[which][...])
        for j in range(NL):
            for c in range(NC):
                bu[i, which * NL + j, TP * c:TP * c + T, :] = res[T * c:T * (c + 1), 128 * j:128 * (j + 1)]

    kvacc[...] = jnp.zeros(kvacc.shape, f32)
    hst[...] = jnp.zeros(hst.shape, f32)
    w2[...] = jnp.zeros(w2.shape, f32)
    for c in (c_lre, c_lim, c_ldt, c_dsk, c_wphi):
        c.wait()

    l_re = lre[...].reshape(1, D).astype(f32)
    l_im = lim[...].reshape(1, D).astype(f32)
    dt = jnp.exp(ldt[...].reshape(1, D).astype(f32)).astype(bf16).astype(f32)
    dvec[...] = jnp.broadcast_to(dsk[...].reshape(1, D).astype(f32), (8, D))
    zr = dt * l_re
    zi = dt * l_im
    sub = lax.broadcasted_iota(i32, (8, D), 0)
    n = (sub + 1).astype(f32)
    mag = jnp.exp(n * zr)
    pr = mag * jnp.cos(n * zi)
    pi = mag * jnp.sin(n * zi)
    a_re = pr[0:1]
    a_im = pi[0:1]
    tabs[8] = jnp.broadcast_to(a_re, (8, D))
    tabs[9] = jnp.broadcast_to(a_im, (8, D))
    a8r = jnp.broadcast_to(pr[7:8], (8, D))
    a8i = jnp.broadcast_to(pi[7:8], (8, D))
    den = l_re * l_re + l_im * l_im
    nr = a_re - 1.0
    s_r = jnp.broadcast_to(2.0 * (nr * l_re + a_im * l_im) / den, (8, D))
    s_i = jnp.broadcast_to(2.0 * (a_im * l_re - nr * l_im) / den, (8, D))
    tabs[10] = s_r
    tabs[11] = s_i
    for q in range(T // 8):
        tr, ti = _cmul(pr, pi, s_r, s_i)
        pwre[8 * q:8 * q + 8, :] = tr
        pwim[8 * q:8 * q + 8, :] = ti
        if q + 1 < T // 8:
            pr, pi = _cmul(pr, pi, a8r, a8i)
    b1r = jnp.broadcast_to(pr[7:8], (8, D))
    b1i = jnp.broadcast_to(pi[7:8], (8, D))
    b2r, b2i = _cmul(b1r, b1i, b1r, b1i)
    b4r, b4i = _cmul(b2r, b2i, b2r, b2i)
    for k, (vr, vi, lo, hi) in enumerate(((b1r, b1i, 0, 1), (b1r, b1i, 1, 8), (b2r, b2i, 2, 8), (b4r, b4i, 4, 8))):
        keep = (sub >= lo) & (sub < hi)
        tabs[2 * k] = jnp.where(keep, vr, 0.0)
        tabs[2 * k + 1] = jnp.where(keep, vi, 0.0)

    for d in range(DH):
        w2[pl.ds(24 * d, DH), :] = wphi[d].astype(f32)
    hrow = lax.broadcasted_iota(i32, (H, D), 0)
    ccol = lax.broadcasted_iota(i32, (H, D), 1)
    hsel = jnp.where(((ccol * 3277) >> 16) == hrow, 1.0, 0.0).astype(bf16)
    r2 = _nn(w2[...].astype(bf16), hsel)
    c8 = lax.broadcasted_iota(i32, (24, D), 1)
    h8 = (c8 * 3277) >> 16
    d8 = c8 - DH * h8
    wpt = jnp.zeros((24, D), f32)
    for d in range(DH):
        wpt = wpt + jnp.where(d8 == d, r2[24 * d:24 * (d + 1)], 0.0)
    rr = lax.broadcasted_iota(i32, (48, 24), 0)
    ff = lax.broadcasted_iota(i32, (48, 24), 1)
    e40 = jnp.where((4 * (rr >> 3) + ((rr & 7) >> 1)) == ff, 1.0, 0.0).astype(bf16)

    r40 = _nn(e40, wpt.astype(bf16))
    subp = lax.broadcasted_iota(i32, (8, 128), 0) & 1
    abands = []
    for kt, (r0, r1) in enumerate(BANDS):
        hc = h8[0:8, 128 * kt:128 * (kt + 1)] - subp
        slabs = []
        for q in range(r0 // 8, r1 // 8):
            slabs.append(jnp.where(hc == 2 * (q // 5), r40[8 * (q % 5):8 * (q % 5) + 8, 128 * kt:128 * (kt + 1)], 0.0))
        abands.append(jnp.concatenate(slabs, 0).astype(bf16))

    c_bre.wait()
    cxb[0].wait()
    bu_proj(0, 0)
    cxb[1].wait()
    bu_proj(1, 0)
    c_bim.wait()
    cxb[2].wait()
    bu_proj(0, 1)
    bu_proj(1, 1)
    bu_proj(2, 0)
    bu_proj(2, 1)
    c_wqkv.wait()
    for i in range(3, LB):
        cxb[i].wait()
    segs = ((0, 112, 0, None), (112, 160, 0, 1), (160, 240, 1, None), (240, 288, 1, 2), (288, 352, 2, None),
            (352, 400, 2, 3), (400, 480, 3, None), (480, 528, 3, 4), (528, 640, 4, None))
    for part in range(2):
        pieces = [_nt(abands[kt], wqkv[:, part * D + 128 * kt: part * D + 128 * (kt + 1)]) for kt in range(5)]
        for r0, r1, ka, kb in segs:
            v = pieces[ka][r0 - BANDS[ka][0]:r1 - BANDS[ka][0]]
            if kb is not None:
                v = v + pieces[kb][r0 - BANDS[kb][0]:r1 - BANDS[kb][0]]
            wt[(part * D + r0) // 2:(part * D + r1) // 2, :] = _pk((v * LOG2E).astype(bf16))
    def wvt(kt, nt):
        def run():
            wt[D + 64 * kt:D + 64 * (kt + 1), 128 * nt:128 * (nt + 1)] = _pk(
                wqkv[128 * nt:128 * (nt + 1), 2 * D + 128 * kt:2 * D + 128 * (kt + 1)].T)
        return run
    tfill = [wvt(kt, nt) for kt in range(5) for nt in range(5)]
    for f in tfill:
        f()
    for i in range(3, LB):
        bu_proj(i, 0)
        bu_proj(i, 1)
    c_cre.wait()
    c_cim.wait()

    def scan(i):
        hr_all, hi_all = [], []
        for j in range(NL):
            ls = slice(128 * j, 128 * (j + 1))
            ar = tabs[8, :, ls]
            ai = tabs[9, :, ls]
            hr = bu[i, j, pl.ds(0, NC, stride=TP), :]
            hi = bu[i, NL + j, pl.ds(0, NC, stride=TP), :]
            for t in range(1, T):
                ur = bu[i, j, pl.ds(t, NC, stride=TP), :]
                ui = bu[i, NL + j, pl.ds(t, NC, stride=TP), :]
                mr, mi = _cmul(ar, ai, hr, hi)
                hr = mr + ur
                hi = mi + ui
                bu[i, j, pl.ds(t, NC, stride=TP), :] = hr
                bu[i, NL + j, pl.ds(t, NC, stride=TP), :] = hi
            inr = hst[0, :, ls]
            ini = hst[1, :, ls]
            mr, mi = _cmul(tabs[0, :, ls], tabs[1, :, ls], inr, ini)
            er = hr + mr
            ei = hi + mi
            for k, sh in ((1, 1), (2, 2), (3, 4)):
                mr, mi = _cmul(tabs[2 * k, :, ls], tabs[2 * k + 1, :, ls],
                               pltpu.roll(er, sh, 0), pltpu.roll(ei, sh, 0))
                er = er + mr
                ei = ei + mi
            subl = lax.broadcasted_iota(i32, (8, 128), 0)
            cinr = jnp.where(subl == 0, inr, pltpu.roll(er, 1, 0))
            cini = jnp.where(subl == 0, ini, pltpu.roll(ei, 1, 0))
            hst[0, :, ls] = jnp.broadcast_to(er[7:8], (8, 128))
            hst[1, :, ls] = jnp.broadcast_to(ei[7:8], (8, 128))
            pr_ = pwre[:, ls]
            pi_ = pwim[:, ls]
            sr_ = jnp.broadcast_to(tabs[10, 0:1, ls], (T, 128))
            si_ = jnp.broadcast_to(tabs[11, 0:1, ls], (T, 128))
            nsr_ = -sr_
            hrs, his = [], []
            for c in range(NC):
                cr = jnp.broadcast_to(cinr[c:c + 1], (T, 128))
                ci = jnp.broadcast_to(cini[c:c + 1], (T, 128))
                mr, mi = _cmul(pr_, pi_, cr, ci)
                lr = bu[i, j, TP * c:TP * c + T, :]
                li = bu[i, NL + j, TP * c:TP * c + T, :]
                hrs.append((lr * sr_ - li * si_) + mr)
                his.append((li * nsr_ - lr * si_) - mi)
            hr_all.append(jnp.concatenate(hrs, 0))
            hi_all.append(jnp.concatenate(his, 0))
        hre = jnp.concatenate(hr_all, 1).astype(bf16)
        him = jnp.concatenate(hi_all, 1).astype(bf16)
        return hre, him

    def phase1(i, with_bu, order=ORDER):
        if with_bu:
            cp_xb(i + LB).wait()
            cp_xa(i).wait()
        xai = xa[i]
        st = {}

        def do_k():
            st['phk'] = _dual_softmax(_nt(_up(wt[D // 2:D, :]), xai))

        def do_q():
            phiq[i] = _dual_softmax(_nt(_up(wt[0:D // 2, :]), xai)).reshape(2 * D, TB).astype(bf16)

        def do_v():
            st['vt'] = _nt(_up(wt[D:3 * D // 2, :]), xai)

        def do_b():
            if with_bu:
                bu_proj(i + LB, 0)

        def do_i():
            if with_bu:
                bu_proj(i + LB, 1)

        def do_z():
            ones8 = jnp.ones((8, TB), f32)
            for g in range(G):
                vaug = jnp.concatenate([st['vt'][40 * g:40 * (g + 1)], ones8], axis=0).astype(bf16)
                kvacc[g] += _nt(vaug, st['phk'][g].reshape(80, TB).astype(bf16))

        def do_s():
            st['h'] = scan(i)

        def do_c():
            hre, him = st['h']
            y = _nt(hre, cre[...]) + _nt(him, cim[...])
            ob[i] = y + xb[i].astype(f32) * dvec[0:1, :]

        def do_d():
            pltpu.make_async_copy(ob.at[i], out_hbm.at[0, pl.ds(i * TB, TB), pl.ds(D, D)], sem_ob.at[i]).start()

        for ch in order:
            dict(k=do_k, q=do_q, v=do_v, b=do_b, i=do_i, z=do_z, s=do_s, c=do_c, d=do_d)[ch]()

    NW = NB - LB
    def run(lo, hi, with_bu):
        lax.fori_loop(lo, hi, lambda i, c: (phase1(i, with_bu), c)[1], 0)
    run(0, NW, True)
    for k in range(NW, NB):
        cxa[k].wait()
    c_wo.wait()
    run(NW, NB - 1, False)
    phase1(NB - 1, False, 'kqvsczd')

    r3 = lax.broadcasted_iota(i32, (G, 48, 80), 1)
    c3 = lax.broadcasted_iota(i32, (G, 48, 80), 2)
    hh_row = jnp.where(r3 < 40, jnp.where(r3 >= 20, 1, 0), jnp.where(r3 >= 44, 1, 0))
    kvb[...] = jnp.where(hh_row == (c3 & 1), kvacc[...], 0.0).astype(bf16)

    def numpart(i):
        os_ = []
        for g in range(G):
            r = _nn(kvb[g], phiq[i, 80 * g:80 * (g + 1), :])
            rd = _rcp(r[40:48] + 1e-6)
            r0 = jnp.broadcast_to(rd[0:1], (8, TB))
            r1 = jnp.broadcast_to(rd[4:5], (8, TB))
            os_.append(r[0:40] * jnp.concatenate([r0, r0, rd, r1, r1], 0))
        return jnp.concatenate(os_, 0).astype(bf16)

    ot = numpart(0)
    for i in range(NB):
        ot_next = numpart(i + 1) if i + 1 < NB else None
        oa[i] = lax.dot_general(ot, wo[...], (((0,), (0,)), ((), ())), preferred_element_type=f32)
        pltpu.make_async_copy(oa.at[i], out_hbm.at[0, pl.ds(i * TB, TB), pl.ds(0, D)], sem_oa.at[i]).start()
        ot = ot_next

    for i in range(NB):
        pltpu.make_async_copy(ob.at[i], out_hbm.at[0, pl.ds(i * TB, TB), pl.ds(D, D)], sem_ob.at[i]).wait()
        pltpu.make_async_copy(oa.at[i], out_hbm.at[0, pl.ds(i * TB, TB), pl.ds(0, D)], sem_oa.at[i]).wait()


@jax.jit
def pallas_concat_heads__linear_kernel_hedgehog__ssm_conv_s5__prompt_kernel(A_x, A_wqkv, A_w_phi, A_wo, B_x, B_Lambda_re, B_Lambda_im, B_B_re, B_B_im,
           B_C_re, B_C_im, B_log_dt, B_Dskip):
    any_spec = pl.BlockSpec(memory_space=pl.ANY)
    V = pltpu.VMEM
    scratch = [
        V((NB, TB, D), bf16), V((NB, TB, D), bf16), V((D, 3 * D), bf16), V((DH, DH, H), bf16),
        V((D, D), bf16), V((D, D), bf16), V((D, D), bf16), V((D, D), bf16), V((D, D), bf16),
        V((D,), bf16), V((D,), bf16), V((D,), bf16), V((D,), bf16),
        V((24 * DH, H), f32), V((3 * D // 2, D), u32),
        V((12, 8, D), f32), V((T, D), f32), V((T, D), f32), V((8, D), f32),
        V((NB, 2 * D, TB), bf16), V((G, 48, 80), f32), V((G, 48, 80), bf16),
        V((NB, 2 * NL, NC * TP, 128), f32), V((2, 8, D), f32),
        V((NB, TB, D), f32), V((NB, TB, D), f32),
        pltpu.SemaphoreType.DMA((11 + 2 * NB,)),
        pltpu.SemaphoreType.DMA((NB,)), pltpu.SemaphoreType.DMA((NB,)),
    ]
    return pl.pallas_call(
        _kernel,
        in_specs=[any_spec] * 13,
        out_specs=any_spec,
        out_shape=jax.ShapeDtypeStruct((1, S, 2 * D), f32),
        scratch_shapes=scratch,
        compiler_params=pltpu.CompilerParams(vmem_limit_bytes=110 * 2 ** 20),
    )(A_x.reshape(NB, TB, D), A_wqkv, jnp.transpose(A_w_phi, (1, 2, 0)), A_wo, B_x.reshape(NB, TB, D),
      B_Lambda_re, B_Lambda_im, B_B_re, B_B_im, B_C_re, B_C_im, B_log_dt, B_Dskip)
```
